```python
import jax
import jax.numpy as jnp

def _softmax(x, axis=-1):
    return jax.nn.softmax(x, axis=axis)
def _gelu(x):
    return jax.nn.gelu(x, approximate=True)
def _silu(x):
    return jax.nn.silu(x)
def _sigmoid(x):
    return jax.nn.sigmoid(x)
def _layernorm(x, axis=-1, eps=1e-5):
    m = jnp.mean(x, axis=axis, keepdims=True)
    v = jnp.var(x, axis=axis, keepdims=True)
    return (x - m) / jnp.sqrt(v + eps)
def _scatter_add(tgt, idx, src, axis=0):
    return tgt.at[idx].add(src)
def _segment_sum(src, seg, n):
    return jax.ops.segment_sum(src, seg, n)
class _Rng:
    def __init__(self, key):
        self._k = key
    def _next(self):
        self._k, sub = jax.random.split(self._k)
        return sub
    def normal(self, shape):
        return jax.random.normal(self._next(), shape, dtype=jnp.bfloat16)
    def randint(self, lo, hi, shape):
        return jax.random.randint(self._next(), shape, lo, hi, dtype=jnp.int32)
    def uniform(self, shape, lo=0.0, hi=1.0):
        return jax.random.uniform(self._next(), shape, jnp.bfloat16, lo, hi)
    def permutation(self, n):
        return jax.random.permutation(self._next(), n)


kernel_name = 'sequential_preLN__softmax_full_mha__glu_gated_geglu__prompt'

def _fwd_setup_inputs():
    _rng = _Rng(jax.random.key(int.from_bytes(__import__("os").urandom(4), "little")))
    _w = (lambda a: (lambda t: t.astype(jnp.bfloat16) if jnp.issubdtype(t.dtype, jnp.floating) else t)(jnp.asarray(a)))
    def _A_setup():
        B, S, D = 1, 2048, 640
        return {
            "x": _w((lambda *s: _rng.normal(s) * 0.05)(B, S, D)),
            "wqkv": _w((lambda *s: _rng.normal(s) * 0.05)(D, 3 * D)),
            "wo": _w((lambda *s: _rng.normal(s) * 0.05)(D, D)),
        }
    _A_in = _A_setup()

    def _B_setup():
        B, S, Dm, Df = 1, 2048, 640, 1536
        return {
            "x": _w((lambda *s: _rng.normal(s) * 0.05)(B, S, Dm)),
            "w_gate": _w((lambda *s: _rng.normal(s) * 0.05)(Dm, Df) * (Dm ** -0.5)),
            "w_up": _w((lambda *s: _rng.normal(s) * 0.05)(Dm, Df) * (Dm ** -0.5)),
            "w_down": _w((lambda *s: _rng.normal(s) * 0.05)(Df, Dm) * (Df ** -0.5)),
        }
    _B_in = _B_setup()

    return {
        "A_x": _A_in["x"],
        "A_wqkv": _A_in["wqkv"],
        "A_wo": _A_in["wo"],
        "B_x": _B_in["x"],
        "B_w_gate": _B_in["w_gate"],
        "B_w_up": _B_in["w_up"],
        "B_w_down": _B_in["w_down"],
    }

def _fwd_reference(A_x, A_wqkv, A_wo, B_x, B_w_gate, B_w_up, B_w_down):
    def _A_ref(x, wqkv, wo):
        B, S, D = x.shape
        H = 32; Dh = D // H
        qkv = (lambda x, *d: x.transpose(*d))((x @ wqkv).reshape(B, S, 3, H, Dh), 2, 0, 3, 1, 4)
        q, k, v = qkv[0], qkv[1], qkv[2]
        scale = Dh ** -0.5
        scores = jnp.einsum("bhqd,bhkd->bhqk", q, k) * scale
        p = _softmax(scores, axis=-1)
        o = jnp.einsum("bhqk,bhkd->bhqd", p, v)
        return (lambda x, *d: x.transpose(*d))(o, 0, 2, 1, 3).reshape(B, S, D) @ wo

    def _B_ref(x, w_gate, w_up, w_down):
        g = jnp.einsum("bsd,df->bsf", x, w_gate)
        u = jnp.einsum("bsd,df->bsf", x, w_up)
        h = _gelu(g) * u
        return jnp.einsum("bsf,fd->bsd", h, w_down)

    x = A_x
    h = x + _A_ref(_layernorm(x, axis=-1), A_wqkv, A_wo)
    h2 = h + _B_ref(_layernorm(h, axis=-1), B_w_gate, B_w_up, B_w_down)
    return h2


def setup_inputs():
    _inp = _fwd_setup_inputs()
    _gk = jax.random.fold_in(jax.random.key(int.from_bytes(__import__("os").urandom(4), "little")), 2**31 - 1)
    _shapes = [[1, 2048, 640]]
    _dtypes = ['bfloat16']
    _gks = jax.random.split(_gk, len(_shapes))
    _gs = [jax.random.normal(k, s, dtype=jnp.dtype(d)) * 0.05 for k, s, d in zip(_gks, _shapes, _dtypes)]
    _inp["grad_out"] = _gs[0]
    return _inp

def reference(A_x, A_wqkv, A_wo, B_w_gate, B_w_up, B_w_down, B_x, grad_out):
    _const = dict(B_x=B_x)
    def _f(*_d):
        return _fwd_reference(**{'A_x': _d[0], 'A_wqkv': _d[1], 'A_wo': _d[2], 'B_w_gate': _d[3], 'B_w_up': _d[4], 'B_w_down': _d[5], **_const})
    _out, _vjp = jax.vjp(_f, A_x, A_wqkv, A_wo, B_w_gate, B_w_up, B_w_down)
    _grads = _vjp(grad_out)
    _out0 = jnp.asarray(_out)
    return (_out0, *[jnp.asarray(_g) for _g in _grads])
```

```python
import math

import jax
import jax.numpy as jnp
from jax import lax
import jax.experimental.pallas as pl
import jax.experimental.pallas.tpu as pltpu

S, D, H, DH, DF = 2048, 640, 32, 20, 1536
TQ = 256
NQB = S // TQ
NQUAD = H // 4
UF = 2
UB = 2
TC = 256
NCH = S // TC
NB = NQUAD // UB
FC = DF // NB
FW = 256
NPA = 4
NPB = 4
FK = 1024
EPS = 1e-5
SCALE = DH ** -0.5
LOG2E = 1.4426950408889634
LN2 = 0.6931471805599453
GELU_C = math.sqrt(2.0 / math.pi)
GELU_A = 0.044715
M_OFF = 32.0
M_LIM = 48.0
_OFF = (0, 4, 0, 4)

bf = jnp.bfloat16
f32 = jnp.float32
u32 = jnp.uint32
_NN = (((1,), (0,)), ((), ()))
_NT = (((1,), (1,)), ((), ()))


def _pk(x):
    return pltpu.bitcast(x, u32)


def _up(x):
    return pltpu.bitcast(x, bf)


def _dot(a, b):
    return lax.dot_general(a, b, _NN, preferred_element_type=f32)


def _dot_nt(a, b):
    return lax.dot_general(a, b, _NT, preferred_element_type=f32)


def _asm(rs):
    return jnp.concatenate([rs[r][_OFF[r]:_OFF[r] + DH] for r in range(4)], axis=0)


def _win24(ref, base, j, r, cols):
    w = _up(ref[pl.ds(pl.multiple_of(base + 40 * j + 8 * r, 8), 16), cols]).astype(f32)
    return w[0:24] if r < 2 else w[8:32]


def _ln_stats(v):
    mu = jnp.mean(v, axis=-1, keepdims=True)
    c = v - mu
    var = jnp.mean(c * c, axis=-1, keepdims=True)
    r = lax.rsqrt(var + EPS)
    return c * r, r


def _ln_bwd(dn, n, r):
    return r * (dn - jnp.mean(dn, axis=-1, keepdims=True)
                - n * jnp.mean(dn * n, axis=-1, keepdims=True))


def _acc(ref, idx, first, val, stage=None, stage_idx=None):
    new = val + jnp.where(first, 0.0, ref[idx])
    ref[idx] = new
    if stage is not None:
        stage[idx if stage_idx is None else stage_idx] = new.astype(bf)


def _head_geom(j, r):
    w0 = jnp.minimum(40 * j, (D - 128) // 2)
    return pl.multiple_of(w0, 8), 40 * j + (DH // 2) * r - w0


def _masked_window(ref, w0, lo, cols):
    win = ref[pl.ds(w0, 64), cols]
    it = lax.broadcasted_iota(jnp.int32, win.shape, 0)
    keep = jnp.logical_and(it >= lo, it < lo + DH // 2)
    return _up(jnp.where(keep, win, jnp.zeros_like(win)))


def _store_head_windows(dst, src, heads=range(H)):
    for h in heads:
        w0 = min(40 * (h // 4), (D - 128) // 2)
        lo = (DH // 2) * h - w0
        t0, t1 = lo // 8 * 8, (lo + DH // 2 + 7) // 8 * 8
        it = lax.broadcasted_iota(jnp.int32, (t1 - t0, TQ), 0) + t0
        win = src(w0 + t0, w0 + t1)
        dst[h, t0:t1, :] = jnp.where(jnp.logical_and(it >= lo, it < lo + DH // 2), win, jnp.zeros_like(win))


def _kernel(x_hbm, wqkv_hbm, wo_hbm, wg_hbm, wu_hbm, wd_hbm, dy_hbm,
            h2_hbm, dx_hbm, dwqkv_hbm, dwo_hbm, dwg_hbm, dwu_hbm, dwd_hbm,
            x_v, dy_v, wqkv_v, wo_v, wg_v, wu_v, wd_v,
            qkvT, ktok, vtok, n1T, n1a, n1b, m_v, nmax, kq,
            p0, p1, p2, p3, oT, lsum, dof_v, w1_v, w2_v, delta_v, hhT_v, seg_v, vbuf, oTb_v, dhb_v,
            dqkv, dh_v, dwo_a, dwg_a, dwu_a, dwd_a,
            n2b_v, n2T_v, dhh_v, dg_v, du_v, hh_v, h_v,
            h2_s, dwqkv_s, dwo_s, dwg_s, dwu_s, dwd_s,
            sem_in, sem_x, sem_out, sem_w):
    P = (p0, p1, p2, p3)

    def x_copy(t):
        rows = pl.ds(pl.multiple_of(t * TC, TC), TC)
        return pltpu.make_async_copy(x_hbm.at[rows], x_v.at[rows], sem_x.at[t])

    def wq_copy(p):
        cols = slice(p * D, (p + 1) * D)
        return pltpu.make_async_copy(wqkv_hbm.at[:, cols], wqkv_v.at[:, cols], sem_in.at[p])

    def fcols(k):
        return slice(k * FC, (k + 1) * FC)

    in_copies = [pltpu.make_async_copy(s, d, sem_in.at[3 + n]) for n, (s, d) in enumerate(
        [(wd_hbm, wd_v), (dy_hbm, dy_v), (wo_hbm, wo_v), (wg_hbm, wg_v), (wu_hbm, wu_v)])]
    x_copy(0).start()
    wq_copy(0).start()

    seg_v[...] = _pk((lax.broadcasted_iota(jnp.int32, (H, 8 * H), 1) >> 3
                      == lax.broadcasted_iota(jnp.int32, (H, 8 * H), 0)).astype(bf))

    nmax[...] = jnp.zeros_like(nmax)

    def zero_windows(h, _):
        w1_v[h] = jnp.zeros((64, TQ), u32)
        w2_v[h] = jnp.zeros((64, TQ), u32)
        return 0

    lax.fori_loop(0, H, zero_windows, 0)

    def ln1(k, dst):
        rows = pl.ds(pl.multiple_of(k * 128, 128), 128)
        n, _ = _ln_stats(x_v[rows, :].astype(f32))
        nb = n.astype(bf)
        dst[...] = _pk(nb)
        n1T[:, rows] = _pk(nb.T)

    def post(part, yb, k):
        cols = pl.ds(pl.multiple_of(k * 128, 128), 128)
        yT = yb.T
        qkvT[part * (D // 2):(part + 1) * (D // 2), cols] = _pk(yT)
        if part > 0:
            tok = ktok if part == 1 else vtok
            yp = _pk(yb)
            lane = lax.broadcasted_iota(jnp.int32, (64, 128), 1)
            for q in range(NQUAD):
                g, sh = divmod(min(80 * q, D - 128), 128)
                w = yp[:, 128 * g:128 * (g + 1)]
                if sh:
                    w = jnp.where(lane >= sh, w, yp[:, 128 * (g + 1):128 * (g + 2)])
                    w = pltpu.roll(w, 128 - sh, 1)
                tok[q, pl.ds(pl.multiple_of(k * 64, 64), 64), :] = w
        if part < 2:
            yf = yT.astype(f32)
            sq = yf * yf
            low = lax.broadcasted_iota(jnp.int32, (8, 128), 0) < 4
            parts = []
            for h in range(H):
                a = DH * h // 8 * 8
                edge = jnp.where(low, 0.0, sq[a:a + 8]) if h % 2 else jnp.where(low, sq[a + 16:a + 24], 0.0)
                a += 8 * (h % 2)
                parts.append(sq[a:a + 8] + sq[a + 8:a + 16] + edge)
            nrm = _dot(_up(seg_v[...]), jnp.concatenate(parts, axis=0).astype(bf))
            nmax[part] = jnp.maximum(nmax[part], nrm)
            if part == 0:
                m_v[:, cols] = nrm

    def qscale(y):
        return (y * (SCALE * LOG2E)).astype(bf)

    x_copy(0).wait()

    def ln1_first(k, _):
        n, _ = _ln_stats(x_v[pl.ds(pl.multiple_of(k * 32, 32), 32), :].astype(f32))
        n1a[pl.ds(pl.multiple_of(k * 16, 16), 16), :] = _pk(n.astype(bf))
        return 0

    lax.fori_loop(0, 4, ln1_first, 0)
    wq_copy(1).start()
    wq_copy(0).wait()
    qa = qscale(_dot(_up(n1a[...]), wqkv_v[:, 0:D]))
    n1T[:, 0:128] = _pk(_up(n1a[...]).T)
    ln1(1, n1b)
    qb = qscale(_dot(_up(n1b[...]), wqkv_v[:, 0:D]))
    wq_copy(2).start()
    x_copy(1).start()
    wq_copy(1).wait()
    ka = _dot(_up(n1a[...]), wqkv_v[:, D:2 * D]).astype(bf)
    kb = _dot(_up(n1b[...]), wqkv_v[:, D:2 * D]).astype(bf)
    post(0, qa, 0)
    post(0, qb, 1)
    wq_copy(2).wait()
    x_copy(1).wait()
    for t in range(2, NCH):
        x_copy(t).start()
    ya = _dot(_up(n1a[...]), wqkv_v[:, 2 * D:3 * D])
    yb = _dot(_up(n1b[...]), wqkv_v[:, 2 * D:3 * D])
    post(1, ka, 0)
    post(1, kb, 1)
    ln1(2, n1a)
    post(2, ya.astype(bf), 0)
    vbuf[...] = _pk(yb.astype(bf))

    def q_windows(j, cols):
        for r in range(4):
            w0, lo = _head_geom(j, r)
            t0 = pl.multiple_of(jnp.minimum((lo >> 3) << 3, 40), 8)
            win = qkvT[pl.ds(pl.multiple_of(w0 + t0, 8), 24), cols]
            it = lax.broadcasted_iota(jnp.int32, win.shape, 0)
            keep = jnp.logical_and(it >= lo - t0, it < lo - t0 + DH // 2)
            w1_v[4 * j + r, pl.ds(t0, 24), :] = jnp.where(keep, win, jnp.zeros_like(win))


    def phase_a(t, _):
        @pl.when(t + 1 < NCH)
        def _():
            x_copy(t + 1).wait()

        @pl.when(t == 2)
        def _():
            for c in in_copies:
                c.start()

        q_windows(t, slice(0, TQ))

        ya = _dot(_up(n1a[...]), wqkv_v[...])
        post(2, _up(vbuf[...]), 2 * t - 1)
        ln1(2 * t + 1, n1b)
        yb = _dot(_up(n1b[...]), wqkv_v[...])
        ln1(jnp.minimum(2 * t + 2, 2 * NCH - 1), n1a)
        for hf, y in enumerate((ya, yb)):
            post(0, qscale(y[:, 0:D]), 2 * t + hf)
            post(1, y[:, D:2 * D].astype(bf), 2 * t + hf)
        post(2, ya[:, 2 * D:3 * D].astype(bf), 2 * t)
        vbuf[...] = _pk(yb[:, 2 * D:3 * D].astype(bf))
        return 0

    lax.fori_loop(1, NCH, phase_a, 0)
    post(2, _up(vbuf[...]), 2 * NCH - 1)
    q_windows(0, slice(0, TQ))

    kmax = jnp.max(nmax[1], axis=1, keepdims=True) * (1.02 * 1.02)
    kq[...] = jnp.broadcast_to(kmax, kq.shape)
    bound_max = jnp.sqrt(jnp.max(jnp.max(nmax[0], axis=1, keepdims=True) * kmax))
    exact = jnp.logical_not(bound_max <= M_LIM)

    @pl.when(exact)
    def _():
        def head(n, _):
            cols = pl.ds(pl.multiple_of((n >> 5) * TQ, TQ), TQ)
            h = n & (H - 1)
            w0, lo = _head_geom(h >> 2, h & 3)
            w = _masked_window(qkvT, w0, lo, cols)

            def chunk(c, mx):
                kc = ktok[h >> 2, pl.ds(pl.multiple_of(c * 64, 64), 64), :]
                return jnp.maximum(mx, jnp.max(_dot(_up(kc), w), axis=0, keepdims=True))

            mx = lax.fori_loop(0, S // 128, chunk, jnp.full((1, TQ), -jnp.inf, f32))
            it = lax.broadcasted_iota(jnp.int32, (H, TQ), 0)
            m_v[:, cols] = jnp.where(it == h, mx, m_v[:, cols])
            return 0

        lax.fori_loop(0, NQB * H, head, 0)

    def h2_copy(i):
        return pltpu.make_async_copy(h2_s, h2_hbm.at[pl.ds(pl.multiple_of(i * TQ, TQ), TQ)], sem_out.at[0])

    def attn_fwd(i):
        cols = pl.ds(pl.multiple_of(i * TQ, TQ), TQ)
        TK = 128
        NC = S // TK

        def body(jj, _):
            ms, accs = {}, {}

            def do_s(u, c):
                j = jj * UF + u
                for r in range(4):
                    if c == 0:
                        row = pl.ds(4 * j + r, 1)
                        mv = m_v[row, cols]
                        ms[r] = jnp.where(exact, mv, jnp.sqrt(mv * kq[row, :]) - M_OFF)
                    ks = slice(c * (TK // 2), (c + 1) * (TK // 2))
                    sT = _dot(_up(ktok[j, ks, :]), _up(w1_v[4 * j + r]))
                    P[r][j, ks, :] = _pk(jnp.exp2(sT - ms[r]).astype(bf))

            def do_o(u, c):
                j = jj * UF + u
                for r in range(4):
                    v = _win24(qkvT, D, j, r, slice(c * TK, (c + 1) * TK))
                    it = lax.broadcasted_iota(jnp.int32, v.shape, 0)
                    v = jnp.where(it == (0 if r % 2 else 23), 1.0, v)
                    t = _dot(v, _up(P[r][j, c * (TK // 2):(c + 1) * (TK // 2), :]))
                    accs[r] = t if c == 0 else t + accs[r]
                if c == NC - 1:
                    ls = [accs[r][0:1] if r % 2 else accs[r][23:24] for r in range(4)]
                    oT[pl.ds(pl.multiple_of(80 * j, 16), 80), :] = _asm([accs[r] for r in range(4)])
                    lsum[j] = jnp.concatenate(ls + ls, axis=0)

            steps = [(u, c) for u in range(UF) for c in range(NC)]

            def fill(k):
                blk = pl.ds(pl.multiple_of(jj * FW, FW), FW)
                rr = pl.ds(pl.multiple_of(i * TQ + k * (TQ // 2), TQ // 2), TQ // 2)
                dhh_v[k * (TQ // 2):(k + 1) * (TQ // 2), blk] = _dot_nt(dy_v[rr, :], wd_v[blk, :])

            N = len(steps)
            for n in range(N + 2):
                if n < N:
                    do_s(*steps[n])
                if n == N - 1:
                    fill(0)
                    fill(1)
                if n >= 2:
                    do_o(*steps[n - 2])
            return 0

        lax.fori_loop(0, NQUAD // UF, body, 0)

    def middle(i):
        rows = pl.ds(pl.multiple_of(i * TQ, TQ), TQ)
        dyb = dy_v[rows, :]
        c0 = NB * FW
        c1 = (c0 + DF) // 2
        dhh_v[:, c0:c1] = _dot_nt(dyb, wd_v[c0:c1, :])

        def row_scale():
            it80 = lax.broadcasted_iota(jnp.int32, (80, TQ), 0)
            lis = [1.0 / lsum[j] for j in range(NQUAD)]
            return lis, jnp.concatenate(
                [jnp.where(it80 < 40, jnp.where(it80 < 20, li[0:1], li[1:2]),
                           jnp.where(it80 < 60, li[2:3], li[3:4])) for li in lis], axis=0)

        oTb = (oT[...] * row_scale()[1]).astype(bf)
        oTp = _pk(oTb)
        for j in range(NQUAD):
            oTb_v[j, 0:40, :] = oTp[40 * j:40 * (j + 1)]
        ob = oTb.T
        RP = TQ // NPA
        hs, r2s, n2s = [], [], []
        for k in range(NPA):
            rk = pl.ds(pl.multiple_of(i * TQ + k * RP, RP), RP)
            hs.append(x_v[rk, :].astype(f32) + _dot(ob[k * RP:(k + 1) * RP], wo_v[...]))
            n2, r2 = _ln_stats(hs[k])
            n2s.append(n2.astype(bf))
            r2s.append(r2)
            n2b_v[k * (RP // 2):(k + 1) * (RP // 2), :] = _pk(n2s[k])
        dhh_v[:, c1:DF] = _dot_nt(dyb, wd_v[c1:DF, :])
        h = jnp.concatenate(hs, axis=0)
        r2 = jnp.concatenate(r2s, axis=0)
        n2b = jnp.concatenate(n2s, axis=0)
        n2T_v[...] = _pk(n2b.T)

        def gate_up(s):
            return _dot(_up(n2b_v[...]), wg_v[:, fcols(s)]), _dot(_up(n2b_v[...]), wu_v[:, fcols(s)])

        gu = [gate_up(0)]
        hhs = []
        dn2 = None
        for s in range(NB):
            if s + 1 < NB:
                gu.append(gate_up(s + 1))
            g, u = gu[s]
            dhh = dhh_v[:, fcols(s)]
            g2 = g * g
            t = jnp.tanh(GELU_C * g * (1.0 + GELU_A * g2))
            hp = 0.5 * (1.0 + t)
            gel = g * hp
            dgel = hp + (0.5 * GELU_C) * g * (1.0 - t * t) * (1.0 + (3.0 * GELU_A) * g2)
            hhs.append((gel * u).astype(bf))
            hhT_v[s] = _pk(hhs[s].T)
            dub = (dhh * gel).astype(bf)
            dgb = (dhh * u * dgel).astype(bf)
            du_v[s] = _pk(dub)
            dg_v[s] = _pk(dgb)
            if s < NB - 1:
                dn = _dot_nt(dgb, wg_v[:, fcols(s)])
                dn2 = dn if dn2 is None else dn + dn2
                dn2 = _dot_nt(dub, wu_v[:, fcols(s)]) + dn2
            if s * FC < FK:
                w = min(FC, FK - s * FC)
                hh_v[:, s * FC:s * FC + w] = _pk(hhs[s][:, 0:w])
        RP = TQ // NPB
        dhs = []
        for k in range(NPB):
            rs = slice(k * RP, (k + 1) * RP)
            dn = _dot_nt(dgb[rs], wg_v[:, fcols(NB - 1)]) + dn2[rs]
            dn = _dot_nt(dub[rs], wu_v[:, fcols(NB - 1)]) + dn
            n2 = _up(n2b_v[k * (RP // 2):(k + 1) * (RP // 2), :]).astype(f32)
            dh = dyb[rs].astype(f32) + _ln_bwd(dn, n2, r2[rs])
            dh_v[pl.ds(pl.multiple_of(i * TQ + k * RP, RP), RP), :] = dh
            dhs.append(dh.astype(bf))
        hr = jnp.concatenate(hhs[NB - 2:], axis=1)[:, FK - (NB - 2) * FC:]
        fm = (DF - FK) // 2
        h = _dot(hr[:, 0:fm], wd_v[FK:FK + fm, :]) + h
        dhb = jnp.concatenate(dhs, axis=0)
        lis, sc = row_scale()
        dhb_v[...] = _pk(dhb)
        for k in range(NB):
            rs = slice(k * (D // NB), (k + 1) * (D // NB))
            dob = (_dot_nt(wo_v[rs, :], dhb) * sc[rs]).astype(bf)
            dobp = _pk(dob)
            _store_head_windows(w2_v, lambda a, b: dobp[a - rs.start // 2:b - rs.start // 2], range(8 * k, 8 * k + 8))
            dof = dob.astype(f32)
            prod = dof * oT[rs, :]
            for u in range(2):
                j = 2 * k + u
                dl = [jnp.sum(prod[80 * u + DH * r:80 * u + DH * (r + 1)], axis=0, keepdims=True) for r in range(4)]
                delta_v[j] = jnp.concatenate(dl + dl, axis=0) * lis[j]
                dof_v[j, 0:80, :] = dof[80 * u:80 * (u + 1)]
        h_v[...] = _dot(hr[:, fm:], wd_v[FK + fm:DF, :]) + h

    def attn_bwd(i):
        cols = pl.ds(pl.multiple_of(i * TQ, TQ), TQ)
        NH = TQ // 128
        NC = S // 128

        def body(jj, _):
            st = [dict() for _ in range(UB)]
            dss = {}
            dk_acc = [None] * 4
            dv_acc = [None] * 4

            def prep(u):
                j = jj * UB + u
                dl = delta_v[j]
                st[u].update(
                    j=j,
                    delta=[dl[r:r + 1] for r in range(4)],
                    qs=[_win24(qkvT, 0, j, r, cols) for r in range(4)],
                    dos=[dof_v[j, (0, 16, 40, 56)[r]:(0, 16, 40, 56)[r] + 24, :] for r in range(4)],
                    dq=[[None] * 4 for _ in range(NH)],
                )

            def do_dp(u, c, hq):
                if c == 0 and hq == 0:
                    prep(u)
                s_ = st[u]
                hs = slice(hq * 128, (hq + 1) * 128)
                for r in range(4):
                    p = _up(P[r][s_['j'], c * 64:(c + 1) * 64, hs])
                    dp = _dot(_up(vtok[s_['j'], c * 64:(c + 1) * 64, :]), _up(w2_v[4 * s_['j'] + r, :, hs]))
                    dss[(u, c, hq, r)] = (p.astype(f32) * (dp - s_['delta'][r][:, hs])).astype(bf)

            def do_dv(u, c, hq):
                s_ = st[u]
                hs = slice(hq * 128, (hq + 1) * 128)
                for r in range(4):
                    t = _dot_nt(s_['dos'][r][:, hs], _up(P[r][s_['j'], c * 64:(c + 1) * 64, hs]))
                    dv_acc[r] = t if hq == 0 else t + dv_acc[r]
                if hq == NH - 1:
                    rr = pl.ds(pl.multiple_of(2 * D + 80 * s_['j'], 16), 80)
                    _acc(dqkv, (rr, slice(c * 128, (c + 1) * 128)), i == 0, _asm(dv_acc))

            def do_dk(u, c, hq):
                s_ = st[u]
                hs = slice(hq * 128, (hq + 1) * 128)
                for r in range(4):
                    t = _dot_nt(s_['qs'][r][:, hs], dss[(u, c, hq, r)])
                    dk_acc[r] = t if hq == 0 else t + dk_acc[r]
                if hq == NH - 1:
                    rr = pl.ds(pl.multiple_of(D + 80 * s_['j'], 16), 80)
                    _acc(dqkv, (rr, slice(c * 128, (c + 1) * 128)), i == 0, _asm(dk_acc))

            def do_dq(u, c, hq):
                s_ = st[u]
                dq = s_['dq']
                for r in range(4):
                    kw = _win24(qkvT, D // 2, s_['j'], r, slice(c * 128, (c + 1) * 128))
                    t = _dot(kw, dss[(u, c, hq, r)])
                    dq[hq][r] = t if c == 0 else t + dq[hq][r]
                if c == NC - 1 and hq == NH - 1:
                    dqq = jnp.concatenate([_asm(dq[k]) for k in range(NH)], axis=1)
                    dqkv[pl.ds(pl.multiple_of(80 * s_['j'], 16), 80), cols] = dqq * SCALE

            steps = [(u, c, hq) for u in range(UB) for c in range(NC) for hq in range(NH)]
            N = len(steps)

            def fill(k):
                j = jj * UB + k
                lhs = _up(oTb_v[j, 0:40, :])
                _acc(dwo_a, (j, slice(0, 80), slice(None)), i == 0, _dot(lhs, _up(dhb_v[...])),
                     dwo_s, (pl.ds(pl.multiple_of(80 * j, 16), 80), slice(None)))

            for n in range(N + 1):
                if n < N:
                    do_dp(*steps[n])
                    do_dv(*steps[n])
                if n == N // 4:
                    for k in range(2):
                        rr = pl.ds(pl.multiple_of(jj * FC + k * (FC // 2), FC // 2), FC // 2)
                        lhs = _up(hhT_v[jj, k * (FC // 4):(k + 1) * (FC // 4), :])
                        _acc(dwd_a, (rr, slice(None)), i == 0, _dot(lhs, dy_v[cols, :]), dwd_s)
                if n == 0:
                    RP = TQ // NB
                    rr = pl.ds(pl.multiple_of(jj * RP, RP), RP)
                    lhs = _up(hh_v[pl.ds(pl.multiple_of(jj * (RP // 2), RP // 2), RP // 2), :])
                    h2_s[rr, :] = (_dot(lhs, wd_v[0:FK, :]) + h_v[rr, :]).astype(bf)
                if n == N // 2:
                    fs = (slice(None), pl.ds(pl.multiple_of(jj * FC, 128), FC))
                    _acc(dwg_a, jj, i == 0, _dot(_up(n2T_v[...]), _up(dg_v[jj])), dwg_s, fs)
                    _acc(dwu_a, jj, i == 0, _dot(_up(n2T_v[...]), _up(du_v[jj])), dwu_s, fs)
                if n == N:
                    for k in range(UB):
                        fill(k)
                if n >= 1:
                    do_dk(*steps[n - 1])
                    do_dq(*steps[n - 1])
            nxt = pl.ds(pl.multiple_of(jnp.minimum(i + 1, NQB - 1) * TQ, TQ), TQ)
            for u in range(UB):
                q_windows(jj * UB + u, nxt)
            return 0

        lax.fori_loop(0, NQUAD // UB, body, 0)

    def qblock(i, _):
        attn_fwd(i)

        @pl.when(i > 0)
        def _():
            h2_copy(i - 1).wait()

        middle(i)
        attn_bwd(i)
        h2_copy(i).start()
        return 0

    for c in in_copies:
        c.wait()
    lax.fori_loop(0, NQB, qblock, 0)

    w_copies = [pltpu.make_async_copy(s, d, sem_w.at[n]) for n, (s, d) in enumerate(
        [(dwd_s, dwd_hbm), (dwg_s, dwg_hbm), (dwu_s, dwu_hbm), (dwo_s, dwo_hbm)])]
    for c in w_copies:
        c.start()
    RW = D // NCH

    def dw_copy(t):
        rows = pl.ds(pl.multiple_of(t * RW, 16), RW)
        return pltpu.make_async_copy(dwqkv_s.at[rows], dwqkv_hbm.at[rows], sem_w.at[4 + t])

    def dx_copy(t):
        rows = pl.ds(pl.multiple_of(t * TC, TC), TC)
        return pltpu.make_async_copy(dy_v.at[rows], dx_hbm.at[rows], sem_x.at[t])

    def phase_c(t, _):
        blks = [pl.ds(pl.multiple_of(t * TC + hf * 128, 128), 128) for hf in range(TC // 128)]
        dn1T = []
        for cols in blks:
            g = jnp.concatenate([dqkv[0:D, cols].astype(bf), (dqkv[D:2 * D, cols] * LN2).astype(bf),
                                 dqkv[2 * D:3 * D, cols].astype(bf)], axis=0)
            dn1T.append(_dot(wqkv_v[...], g))
        lhs = _up(n1T[pl.ds(pl.multiple_of(t * (RW // 2), 8), RW // 2), :])
        for part in range(3):
            dw = _dot_nt(lhs, dqkv[part * D:(part + 1) * D, :].astype(bf))
            if part == 1:
                dw = dw * LN2
            dwqkv_s[pl.ds(pl.multiple_of(t * RW, 16), RW), part * D:(part + 1) * D] = dw.astype(bf)
        for rows, dn in zip(blks, dn1T):
            n1, r1 = _ln_stats(x_v[rows, :].astype(f32))
            dx = dh_v[rows, :] + _ln_bwd(dn.T, n1, r1)
            dy_v[rows, :] = dx.astype(bf)
        dw_copy(t).start()
        dx_copy(t).start()
        return 0

    lax.fori_loop(0, NCH, phase_c, 0)
    h2_copy(NQB - 1).wait()
    for c in w_copies:
        c.wait()

    def wait_out(t, _):
        dw_copy(t).wait()
        dx_copy(t).wait()
        return 0

    lax.fori_loop(0, NCH, wait_out, 0)


@jax.jit
def pallas_sequential_preLN__softmax_full_mha__glu_gated_geglu__prompt_kernel(
    A_x: jax.Array,
    A_wqkv: jax.Array,
    A_wo: jax.Array,
    B_x: jax.Array,
    B_w_gate: jax.Array,
    B_w_up: jax.Array,
    B_w_down: jax.Array,
    grad_out: jax.Array,
):
    del B_x
    V = pltpu.VMEM
    any_spec = pl.BlockSpec(memory_space=pl.ANY)
    out_shape = (
        jax.ShapeDtypeStruct((S, D), bf), jax.ShapeDtypeStruct((S, D), bf),
        jax.ShapeDtypeStruct((D, 3 * D), bf), jax.ShapeDtypeStruct((D, D), bf),
        jax.ShapeDtypeStruct((D, DF), bf), jax.ShapeDtypeStruct((D, DF), bf),
        jax.ShapeDtypeStruct((DF, D), bf),
    )
    scratch = [
        V((S, D), bf), V((S, D), bf), V((D, 3 * D), bf), V((D, D), bf),
        V((D, DF), bf), V((D, DF), bf), V((DF, D), bf),
        V((3 * D // 2, S), u32), V((NQUAD, S // 2, 128), u32), V((NQUAD, S // 2, 128), u32),
        V((D // 2, S), u32), V((64, D), u32), V((64, D), u32),
        V((H, S), f32), V((2, H, 128), f32), V((H, TQ), f32),
        V((NQUAD, S // 2, TQ), u32), V((NQUAD, S // 2, TQ), u32),
        V((NQUAD, S // 2, TQ), u32), V((NQUAD, S // 2, TQ), u32),
        V((D, TQ), f32), V((NQUAD, 8, TQ), f32), V((NQUAD, 128, TQ), f32),
        V((H, 64, TQ), u32), V((H, 64, TQ), u32), V((NQUAD, 8, TQ), f32),
        V((NB, FC // 2, TQ), u32), V((H // 2, 8 * H), u32), V((64, D), u32),
        V((NQUAD, 48, TQ), u32), V((TQ // 2, D), u32),
        V((3 * D, S), f32), V((S, D), f32),
        V((NQUAD, 96, D), f32), V((NB, D, FC), f32), V((NB, D, FC), f32), V((DF, D), f32),
        V((TQ // 2, D), u32), V((D // 2, TQ), u32), V((TQ, DF), f32),
        V((NB, TQ // 2, FC), u32), V((NB, TQ // 2, FC), u32),
        V((TQ // 2, FK), u32), V((TQ, D), f32),
        V((TQ, D), bf), V((D, 3 * D), bf), V((D, D), bf),
        V((D, DF), bf), V((D, DF), bf), V((DF, D), bf),
        pltpu.SemaphoreType.DMA((8,)), pltpu.SemaphoreType.DMA((NCH,)),
        pltpu.SemaphoreType.DMA((1,)), pltpu.SemaphoreType.DMA((4 + NCH,)),
    ]
    outs = pl.pallas_call(
        _kernel,
        out_shape=out_shape,
        in_specs=[any_spec] * 7,
        out_specs=[any_spec] * 7,
        scratch_shapes=scratch,
        compiler_params=pltpu.CompilerParams(vmem_limit_bytes=126 * 1024 * 1024),
    )(A_x.reshape(S, D), A_wqkv, A_wo, B_w_gate, B_w_up, B_w_down, grad_out.reshape(S, D))
    h2, dx = outs[0].reshape(1, S, D), outs[1].reshape(1, S, D)
    return (h2, dx) + tuple(outs[2:])
```
